```python
import os as _os
_os.environ.setdefault("JAX_PLATFORMS", "cpu")
import jax
import jax.numpy as jnp

def _softmax(x, axis=-1):
    return jax.nn.softmax(x, axis=axis)
def _gelu(x):
    return jax.nn.gelu(x, approximate=True)
def _silu(x):
    return jax.nn.silu(x)
def _sigmoid(x):
    return jax.nn.sigmoid(x)
def _layernorm(x, axis=-1, eps=1e-5):
    m = jnp.mean(x, axis=axis, keepdims=True)
    v = jnp.var(x, axis=axis, keepdims=True)
    return (x - m) / jnp.sqrt(v + eps)
def _scatter_add(tgt, idx, src, axis=0):
    return tgt.at[idx].add(src)
def _segment_sum(src, seg, n):
    return jax.ops.segment_sum(src, seg, n)
class _Rng:
    def __init__(self, key):
        self._k = key
    def _next(self):
        self._k, sub = jax.random.split(self._k)
        return sub
    def normal(self, shape):
        return jax.random.normal(self._next(), shape, dtype=jnp.bfloat16)
    def randint(self, lo, hi, shape):
        return jax.random.randint(self._next(), shape, lo, hi, dtype=jnp.int32)
    def uniform(self, shape, lo=0.0, hi=1.0):
        return jax.random.uniform(self._next(), shape, jnp.bfloat16, lo, hi)
    def permutation(self, n):
        return jax.random.permutation(self._next(), n)


kernel_name = 'concat_heads__sliding_local_dilated__sliding_block__prompt'

def setup_inputs():
    _rng = _Rng(jax.random.key(int.from_bytes(__import__("os").urandom(4), "little")))
    _w = (lambda a: (lambda t: t.astype(jnp.bfloat16) if jnp.issubdtype(t.dtype, jnp.floating) else t)(jnp.asarray(a)))
    def _A_setup():
        B, S, D = 1, 2048, 1024
        return {
            "x": _w((lambda *s: _rng.normal(s) * 0.2)(B, S, D)),
            "wqkv": _w((lambda *s: _rng.normal(s) * 0.2)(D, 3 * D)),
            "wo": _w((lambda *s: _rng.normal(s) * 0.05)(D, D)),
        }
    _A_in = _A_setup()

    def _B_setup():
        B, S, D = 1, 2048, 1024
        return {
            "x": _w((lambda *s: _rng.normal(s) * 0.2)(B, S, D)),
            "wqkv": _w((lambda *s: _rng.normal(s) * 0.2)(D, 3 * D)),
            "wo": _w((lambda *s: _rng.normal(s) * 0.05)(D, D)),
        }
    _B_in = _B_setup()

    return {
        "A_x": _A_in["x"],
        "A_wqkv": _A_in["wqkv"],
        "A_wo": _A_in["wo"],
        "B_x": _B_in["x"],
        "B_wqkv": _B_in["wqkv"],
        "B_wo": _B_in["wo"],
    }

def reference(A_x, A_wqkv, A_wo, B_x, B_wqkv, B_wo):
    def _A_ref(x, wqkv, wo):
        B, S, D = x.shape
        H = 32; Dh = D // H
        W, dil = 8, 2
        qkv = (lambda x, *d: x.transpose(*d))((x @ wqkv).reshape(B, S, 3, H, Dh), 2, 0, 3, 1, 4)
        q, k, v = qkv[0], qkv[1], qkv[2]
        scale = Dh ** -0.5
        pos = jnp.arange(S)
        off = jnp.arange(W) * dil
        idx = pos[:, None] - off[None, :]
        mask = idx >= 0
        idx_c = jnp.where(mask, idx, 0).reshape(-1)
        kg = k[:, :, idx_c, :].reshape(B, H, S, W, Dh)
        vg = v[:, :, idx_c, :].reshape(B, H, S, W, Dh)
        logits = jnp.einsum("bhsd,bhswd->bhsw", q, kg) * scale
        logits = jnp.where(mask[None, None, :, :], logits, -1e9)
        attn = _softmax(logits, axis=-1)
        o = jnp.einsum("bhsw,bhswd->bhsd", attn, vg)
        return (lambda x, *d: x.transpose(*d))(o, 0, 2, 1, 3).reshape(B, S, D) @ wo

    def _B_ref(x, wqkv, wo):
        B, S, D = x.shape
        H = 32; Dh = D // H; W = 256
        qkv = (lambda x, *d: x.transpose(*d))((x @ wqkv).reshape(B, S, 3, H, Dh), 2, 0, 3, 1, 4)
        q, k, v = qkv[0], qkv[1], qkv[2]
        scores = jnp.einsum("bhqd,bhkd->bhqk", q, k) * (Dh ** -0.5)
        idx = jnp.arange(S)
        mask = (idx[:, None] - idx[None, :] >= 0) & (idx[:, None] - idx[None, :] < W)
        scores = jnp.where(mask[None, None], scores, -1e9)
        p = _softmax(scores, axis=-1)
        o = jnp.einsum("bhqk,bhkd->bhqd", p, v)
        return (lambda x, *d: x.transpose(*d))(o, 0, 2, 1, 3).reshape(B, S, D) @ wo

    a = _A_ref(A_x, A_wqkv, A_wo)
    b = _B_ref(B_x, B_wqkv, B_wo)
    return jnp.concatenate([a, b], axis=-1)
```

```python
import functools
import numpy as np
import jax
import jax.numpy as jnp
from jax import lax
from jax.experimental import pallas as pl
from jax.experimental.pallas import tpu as pltpu

S = 2048
D = 1024
H = 32
DH = 32
LOG2E = 1.4426950408889634
QSCALE = float(DH ** -0.5 * LOG2E)
NEG = -1e30
TQ = 256
TO = 512
KPAD = 16
NB = S // 128
f32 = jnp.float32
bf16 = jnp.bfloat16


def _dot(a, b):
    return jnp.dot(a, b, preferred_element_type=f32)


def _dot_nt(a, b):
    return lax.dot_general(a, b, (((1,), (1,)), ((), ())), preferred_element_type=f32)


def _kernel(xa_hbm, wa_hbm, woa_hbm, xb_hbm, wb_hbm, wob_hbm, out_hbm,
            x_v, w_v, wo_v, q_s, k_s, vt_s, o_s, out_v, bias_a, sem_x, sem_w, sem_wo, sem_out):
    x_hbm = (xa_hbm, xb_hbm)
    w_hbm = (wa_hbm, wb_hbm)
    wo_hbm = (woa_hbm, wob_hbm)
    NRB = S // TQ

    def x_copy(br, rb):
        return pltpu.make_async_copy(x_hbm[br].at[0, pl.ds(rb * TQ, TQ), :], x_v.at[br, pl.ds(rb * TQ, TQ), :],
                                     sem_x.at[br * NRB + rb])

    def w_copy(br, c):
        return pltpu.make_async_copy(w_hbm[br].at[:, pl.ds(c * D, D)], w_v.at[br, :, pl.ds(c * D, D)],
                                     sem_w.at[br * 3 + c])

    def wo_copy(br):
        return pltpu.make_async_copy(wo_hbm[br], wo_v.at[br], sem_wo.at[br])

    x_copy(0, 0).start()
    for c in range(3):
        w_copy(0, c).start()
    for rb in range(1, NRB):
        x_copy(0, rb).start()
    x_copy(1, 0).start()
    for c in range(3):
        w_copy(1, c).start()
    for rb in range(1, NRB):
        x_copy(1, rb).start()
    wo_copy(0).start()
    wo_copy(1).start()

    row = lax.broadcasted_iota(jnp.int32, (144, 128), 0)
    col = lax.broadcasted_iota(jnp.int32, (144, 128), 1)
    dd = col - row + 16
    ok = (dd >= 0) & (dd <= 14) & ((dd & 1) == 0)
    bias_a[...] = jnp.where(ok, 0.0, NEG).astype(f32)
    k_s[0, 0:KPAD, :] = jnp.zeros((KPAD, D), bf16)
    vt_s[0, 0] = jnp.zeros((D, 128), bf16)

    def qkv_body(it, carry):
        br = it // NRB
        rb = it % NRB
        pltpu.make_async_copy(xa_hbm.at[0, pl.ds(0, TQ), :], x_v.at[0, pl.ds(0, TQ), :], sem_x.at[it]).wait()

        @pl.when(rb == 0)
        def _():
            for c in range(3):
                pltpu.make_async_copy(wa_hbm.at[:, pl.ds(0, D)], w_v.at[0, :, pl.ds(0, D)], sem_w.at[br * 3 + c]).wait()

        r0 = pl.multiple_of(rb * TQ, TQ)
        xb = x_v[br, pl.ds(r0, TQ), :]
        q = _dot(xb, w_v[br, :, 0:D]) * QSCALE
        q_s[br, pl.ds(r0, TQ), :] = q.astype(bf16)
        k = _dot(xb, w_v[br, :, D:2 * D])
        k_s[br, pl.ds(pl.multiple_of(r0 + KPAD, 16), TQ), :] = k.astype(bf16)
        v = _dot(xb, w_v[br, :, 2 * D:3 * D]).astype(bf16)
        for t in range(TQ // 128):
            vt_s[br, 1 + rb * (TQ // 128) + t] = v[t * 128:(t + 1) * 128, :].T
        return carry

    lax.fori_loop(0, 2 * NRB, qkv_body, 0)

    lane_head = lax.broadcasted_iota(jnp.int32, (128, 128), 1) // DH

    def attn_a_body(i, carry):
        r0 = pl.multiple_of(i * 128, 128)
        for g in range(8):
            ls = slice(g * 128, (g + 1) * 128)
            q = q_s[0, pl.ds(r0, 128), ls]
            kw = k_s[0, pl.ds(pl.multiple_of(r0 + KPAD - 16, 16), 144), ls]
            outs = []
            for h in range(4):
                qm = jnp.where(lane_head == h, q, jnp.zeros_like(q))
                sT = _dot_nt(kw, qm) + bias_a[...]
                halo = jnp.where(i > 0, sT[0:16], NEG)
                sT = jnp.concatenate([halo, sT[16:]], axis=0)
                m = jnp.max(sT, axis=0, keepdims=True)
                p = jnp.exp2(sT - m)
                l = jnp.sum(p, axis=0, keepdims=True)
                pb = jnp.concatenate([jnp.zeros((112, 128), bf16), p.astype(bf16)], axis=0)
                hs = slice((g * 4 + h) * DH, (g * 4 + h + 1) * DH)
                vt = jnp.concatenate([vt_s[0, i, hs, :], vt_s[0, i + 1, hs, :]], axis=1)
                outs.append(_dot(vt, pb) / l)
            oT = jnp.concatenate(outs, axis=0).astype(bf16)
            o_s[0, pl.ds(r0, 128), ls] = oT.T
        return carry

    lax.fori_loop(0, NB, attn_a_body, 0)

    rowi = lax.broadcasted_iota(jnp.int32, (128, 128), 0)
    coli = lax.broadcasted_iota(jnp.int32, (128, 128), 1)
    le = rowi <= coli

    def attn_b_unit(i, g, nkb):
        ls = slice(g * 128, (g + 1) * 128)
        r0 = pl.multiple_of(i * 128, 128)
        q = q_s[1, pl.ds(r0, 128), ls]
        kw = k_s[1, pl.ds(pl.multiple_of(r0 + KPAD - (nkb - 1) * 128, 16), nkb * 128), ls]
        outs = []
        for h in range(4):
            qm = jnp.where(lane_head == h, q, jnp.zeros_like(q))
            sT = _dot_nt(kw, qm)
            hs = slice((g * 4 + h) * DH, (g * 4 + h + 1) * DH)
            if nkb == 3:
                s0, s1, s2 = sT[0:128], sT[128:256], sT[256:384]
                c = jnp.where(le, s2, s0)
                m = jnp.max(jnp.maximum(c, s1), axis=0, keepdims=True)
                pc = jnp.exp2(c - m)
                p1 = jnp.exp2(s1 - m)
                l = jnp.sum(pc + p1, axis=0, keepdims=True)
                p2 = jnp.where(le, pc, 0.0).astype(bf16)
                p0 = jnp.where(le, 0.0, pc).astype(bf16)
                pb = jnp.concatenate([p0, p1.astype(bf16), p2], axis=0)
            elif nkb == 2:
                s1, s2 = sT[0:128], sT[128:256]
                c = jnp.where(le, s2, NEG)
                m = jnp.max(jnp.maximum(c, s1), axis=0, keepdims=True)
                pc = jnp.exp2(c - m)
                p1 = jnp.exp2(s1 - m)
                l = jnp.sum(pc + p1, axis=0, keepdims=True)
                pb = jnp.concatenate([p1.astype(bf16), pc.astype(bf16)], axis=0)
            else:
                c = jnp.where(le, sT, NEG)
                m = jnp.max(c, axis=0, keepdims=True)
                pc = jnp.exp2(c - m)
                l = jnp.sum(pc, axis=0, keepdims=True)
                pb = pc.astype(bf16)
            vt = jnp.concatenate([vt_s[1, i + 1 - (nkb - 1) + t, hs, :] for t in range(nkb)], axis=1)
            outs.append(_dot(vt, pb) / l)
        oT = jnp.concatenate(outs, axis=0).astype(bf16)
        o_s[1, pl.ds(r0, 128), ls] = oT.T

    for g in range(8):
        attn_b_unit(0, g, 1)
    for g in range(8):
        attn_b_unit(1, g, 2)

    def attn_b_body(i, carry):
        for g in range(8):
            attn_b_unit(i, g, 3)
        return carry

    lax.fori_loop(2, NB, attn_b_body, 0)

    NOB = S // TO
    wo_copy(0).wait()
    wo_copy(1).wait()

    def out_copy(br, rb):
        return pltpu.make_async_copy(out_v.at[br, pl.ds(rb * TO, TO), :],
                                     out_hbm.at[0, pl.ds(rb * TO, TO), pl.ds(br * D, D)],
                                     sem_out.at[br * NOB + rb])

    def out_body(it, carry):
        br = it // NOB
        rb = it % NOB
        r0 = pl.multiple_of(rb * TO, TO)
        out_v[br, pl.ds(r0, TO), :] = _dot(o_s[br, pl.ds(r0, TO), :], wo_v[br]).astype(bf16)
        pltpu.make_async_copy(out_v.at[br, pl.ds(r0, TO), :],
                              out_hbm.at[0, pl.ds(r0, TO), pl.ds(pl.multiple_of(br * D, D), D)],
                              sem_out.at[it]).start()
        return carry

    lax.fori_loop(0, 2 * NOB, out_body, 0)
    for br in range(2):
        for rb in range(NOB):
            out_copy(br, rb).wait()


def _call(A_x, A_wqkv, A_wo, B_x, B_wqkv, B_wo, interpret=False):
    any_spec = pl.BlockSpec(memory_space=pl.ANY)
    return pl.pallas_call(
        _kernel,
        out_shape=jax.ShapeDtypeStruct((1, S, 2 * D), bf16),
        in_specs=[any_spec] * 6,
        out_specs=any_spec,
        scratch_shapes=[
            pltpu.VMEM((2, S, D), bf16),
            pltpu.VMEM((2, D, 3 * D), bf16),
            pltpu.VMEM((2, D, D), bf16),
            pltpu.VMEM((2, S, D), bf16),
            pltpu.VMEM((2, KPAD + S, D), bf16),
            pltpu.VMEM((2, NB + 1, D, 128), bf16),
            pltpu.VMEM((2, S, D), bf16),
            pltpu.VMEM((2, S, D), bf16),
            pltpu.VMEM((144, 128), f32),
            pltpu.SemaphoreType.DMA((2 * (S // TQ),)),
            pltpu.SemaphoreType.DMA((6,)),
            pltpu.SemaphoreType.DMA((2,)),
            pltpu.SemaphoreType.DMA((2 * (S // TO),)),
        ],
        compiler_params=pltpu.CompilerParams(vmem_limit_bytes=100 * 1024 * 1024),
        interpret=interpret,
    )(A_x, A_wqkv, A_wo, B_x, B_wqkv, B_wo)


@jax.jit
def pallas_concat_heads__sliding_local_dilated__sliding_block__prompt_kernel(A_x, A_wqkv, A_wo, B_x, B_wqkv, B_wo):
    return _call(A_x, A_wqkv, A_wo, B_x, B_wqkv, B_wo)
```

```python
import functools
import numpy as np
import jax
import jax.numpy as jnp
from jax import lax
from jax.experimental import pallas as pl
from jax.experimental.pallas import tpu as pltpu

S = 2048
D = 1024
H = 32
DH = 32
LOG2E = 1.4426950408889634
QSCALE = float(DH ** -0.5 * LOG2E)
NEG = float("-inf")
T = 256
NT = S // T
KPAD = 16
NB = S // 128
CW = 256
NCH = 3 * D // CW
L_LO = float(2.0 ** -60)
L_HI = float(2.0 ** 60)
f32 = jnp.float32
bf16 = jnp.bfloat16
u32 = jnp.uint32
DEPTH_A = 3
DEPTH_B = 2
DEPK = 4
PORD = (1, 0, 2)
GROUPS = (1, 1, 2, 3, 5)
ISSUE = (1, 4, 7, 12, 12)
OSPLIT = 2


def _dot(a, b):
    return jnp.dot(a, b, preferred_element_type=f32)


def _dot_nt(a, b):
    return lax.dot_general(a, b, (((1,), (1,)), ((), ())), preferred_element_type=f32)


def _iota(shape, dim):
    return lax.broadcasted_iota(jnp.int32, shape, dim)


def _fold8(x):
    acc = x[0:8]
    for j in range(1, x.shape[0] // 8):
        acc = acc + x[8 * j:8 * j + 8]
    return acc


def _recip(l):
    r = pltpu.reciprocal(l, approx=True)
    return r * (2.0 - l * r)


def _mult(x, m):
    return x if isinstance(x, int) else pl.multiple_of(x, m)


def _kernel(xa_hbm, wa_hbm, woa_hbm, xb_hbm, wb_hbm, wob_hbm, out_hbm,
            x_v, w_v, wo_v, q_s, k_s, vt_s, vsh_s, vprev_s, o_s, out_v, bias_a, zero_s,
            sem_x, sem_wa, sem_wb, sem_wo, sem_out):
    x_hbm = (xa_hbm, xb_hbm)

    def x_copy(br, t):
        r0 = _mult(t * T, T)
        return pltpu.make_async_copy(x_hbm[br].at[0, pl.ds(r0, T), :], x_v.at[br, pl.ds(r0, T), :],
                                     sem_x.at[br * NT + t])

    def wa_copy(c):
        return pltpu.make_async_copy(wa_hbm.at[:, pl.ds(c * CW, CW)], w_v.at[0, :, pl.ds(c * CW, CW)], sem_wa.at[c])

    def wb_copy():
        return pltpu.make_async_copy(wb_hbm, w_v.at[1], sem_wb.at[0])

    def woa_copy(kt, p):
        gg, e = kt // 2, kt % 2
        src = (8 * gg + 2 * p + e) * DH
        return pltpu.make_async_copy(woa_hbm.at[pl.ds(src, DH), :], wo_v.at[0, pl.ds(kt * 128 + p * DH, DH), :],
                                     sem_wo.at[0])

    def wob_copy():
        return pltpu.make_async_copy(wob_hbm, wo_v.at[1], sem_wo.at[1])

    def out_copy(br, t, c=0, n=1):
        r0 = _mult(t * T, T)
        w = D // n
        return pltpu.make_async_copy(out_v.at[br, pl.ds(r0, T), pl.ds(c * w, w)],
                                     out_hbm.at[0, pl.ds(r0, T), pl.ds(br * D + c * w, w)],
                                     sem_out.at[br * NT + t + c])

    chunk_order = [c for part in PORD for c in range(part * D // CW, (part + 1) * D // CW)]
    groups = [g for g in GROUPS]
    starts = [sum(groups[:n]) for n in range(len(groups))]
    issued = [0]

    def issue_upto(k):
        while issued[0] < min(k, NCH):
            wa_copy(chunk_order[issued[0]]).start()
            issued[0] += 1

    x_copy(0, 0).start()
    issue_upto(ISSUE[0])
    x_copy(0, 1).start()

    def wait_chunk(c):
        pos = chunk_order.index(c)
        if pos not in starts:
            return
        n = starts.index(pos)
        if n == 0:
            x_copy(0, 0).wait()
            x_copy(0, 1).wait()
        for cc in chunk_order[pos:pos + groups[n]]:
            wa_copy(cc).wait()
        if n + 1 < len(groups):
            issue_upto(ISSUE[n + 1])
        else:
            x_copy(0, 2).start()
            for kt in range(8):
                for p in range(4):
                    woa_copy(kt, p).start()

    row = _iota((80, 128), 0)
    col = _iota((80, 128), 1) & 63
    dd = col - row + 16
    ok = (dd >= 0) & (dd <= 14) & ((dd & 1) == 0)
    bias_a[1] = jnp.where(ok, 0.0, NEG).astype(f32)
    bias_a[0] = jnp.where(ok & (row >= 16), 0.0, NEG).astype(f32)
    for g in range(8):
        k_s[0, g, 0:KPAD, :] = jnp.zeros((KPAD, 128), bf16)
    vprev_s[...] = jnp.zeros((64, D), f32)
    zero_s[...] = jnp.zeros((8, 128), u32)

    lane_head32 = _iota((32, 128), 1) // DH
    lane_head64 = _iota((64, 128), 1) // DH
    lane_lo = _iota((DH, 128), 1) < 64
    le = _iota((128, 128), 0) <= _iota((128, 128), 1)

    lane16 = _iota((16, 128), 1)
    zero16 = jnp.zeros((16, 128), u32)

    def stack_rows(blocks):
        return pltpu.bitcast(jnp.concatenate([zero16 if b is None else b for b in blocks], axis=0), bf16)

    def head_weights(qt):
        qu = pltpu.bitcast(qt, u32)
        return jnp.concatenate(
            [stack_rows([qu[16 * h:16 * h + 16] if hh == h else None for hh in range(4)]) for h in range(4)], axis=1)

    def proj_tasks(br, t, sh_tile, first=False):
        rows = 2 * T if first else T
        r0 = _mult(t * T, T)
        t0 = t * (T // 128)

        def part(c):
            if first:
                wait_chunk(c)
            return _dot(x_v[br, pl.ds(r0, rows), :], w_v[br, :, c * CW:(c + 1) * CW])

        def v_task(c):
            def run():
                v = part(2 * D // CW + c)
                cs = slice(c * CW, (c + 1) * CW)
                for tt in range(rows // 128):
                    vt_s[br, t0 + tt, cs, :] = v[tt * 128:(tt + 1) * 128, :].T.astype(bf16)
                if sh_tile is not None:
                    vsh_s[sh_tile, cs, :] = jnp.concatenate([vprev_s[:, cs], v[0:64]], axis=0).T.astype(bf16)
                    for tt in range(1, rows // 128):
                        vsh_s[sh_tile + tt, cs, :] = v[tt * 128 - 64:tt * 128 + 64, :].T.astype(bf16)
                    vprev_s[:, cs] = v[rows - 64:rows]
            return run

        def q_task(c):
            def run():
                q = part(c) * QSCALE
                cs = slice(c * CW, (c + 1) * CW)
                for tt in range(rows // 128):
                    q_s[br, t0 + tt, cs, :] = q[tt * 128:(tt + 1) * 128, :].T.astype(bf16)
            return run

        def k_task(c):
            def run():
                k = part(D // CW + c).astype(bf16)
                for g in range(CW // 128):
                    k_s[br, c * CW // 128 + g, pl.ds(_mult(r0 + KPAD, 16), rows), :] = k[:, g * 128:(g + 1) * 128]
            return run

        n = D // CW
        tasks = {0: [q_task(c) for c in range(n)], 1: [k_task(c) for c in range(n)], 2: [v_task(c) for c in range(n)]}
        return [f for p in (PORD if first else (2, 0, 1)) for f in tasks[p]]

    def a_qk(i, s, gg):
        j64 = _mult(i * 128 + s * 64, 64)
        out = []
        for gl in range(2):
            g = 2 * gg + gl
            qu = pltpu.bitcast(q_s[0, i, pl.ds(_mult(g * 128, 128), 128), :], u32)
            kw = k_s[0, g, pl.ds(j64, 80), :]
            tiles = []
            for p in range(2):
                ev = qu[32 * p:32 * p + 16]
                od = qu[32 * p + 16:32 * p + 32]
                if s == 0:
                    od = pltpu.roll(od, 64, axis=1)
                else:
                    ev = pltpu.roll(ev, 64, axis=1)
                blocks = [None] * 4
                blocks[2 * p] = jnp.where(lane16 < 64, ev, zero16)
                blocks[2 * p + 1] = jnp.where(lane16 >= 64, od, zero16)
                tiles.append(stack_rows(blocks))
            out.append(_dot(kw, jnp.concatenate(tiles, axis=1)))
        return out

    def a_sm(sTs, bias, safe):
        ps = []
        for gl in range(2):
            for pp in range(2):
                s = sTs[gl][:, pp * 128:(pp + 1) * 128] + bias
                if safe:
                    s = s - jnp.max(s, axis=0, keepdims=True)
                p = jnp.exp2(s)
                l = jnp.sum(_fold8(p), axis=0, keepdims=True)
                pb = jnp.concatenate([jnp.zeros((48, 128), f32), p], axis=0).astype(bf16)
                ps.append((pb, l))
        return ps

    def a_pv(ps, vt_ref, gg, chk):
        ws = []
        for p in range(4):
            pb, l = ps[p]
            x = _dot(vt_ref[pl.ds(_mult(gg * 256 + p * 64, 64), 64), :], pb)
            w = jnp.where(lane_lo, x[0:32], x[32:64])
            if chk is None:
                w = w / l
            else:
                w = w * _recip(l)
                chk = (jnp.minimum(chk[0], l), jnp.maximum(chk[1], l), chk[2] + _fold8(w))
            ws.append(w)
        return jnp.concatenate(ws, axis=0).T.astype(bf16), chk

    def run_units(n_units, qk, sm, pv, fillers, slots, chk, depth=1):
        fillers = list(fillers)
        sts = [qk(n, None) for n in range(depth)]
        tiles = []
        for n in range(n_units):
            for _ in range(slots[n]):
                if fillers:
                    fillers.pop(0)()
            ps, dep = sm(n, sts[n])
            if n + depth < n_units:
                sts.append(qk(n + depth, dep))
            tile, chk = pv(n, ps, chk)
            tiles.append(tile)
        for f in fillers:
            f()
        return tiles, chk

    def attn_a(t, chk, fillers=(), slots=None):
        units = [(ii, s, gg) for ii in range(2) for gg in range(4) for s in range(2)]

        def qk(n, dep):
            ii, s, gg = units[n]
            return a_qk(t * 2 + ii, s, gg)

        def sm(n, sT):
            ii, s, gg = units[n]
            if s == 0 and ii == 0:
                bias = bias_a[min(t, 1) if isinstance(t, int) else jnp.minimum(t, 1)]
            else:
                bias = bias_a[1]
            return a_sm(sT, bias, False), None

        def pv(n, ps, chk):
            ii, s, gg = units[n]
            i = t * 2 + ii
            vt_ref = vsh_s.at[i] if s == 0 else vt_s.at[0, i]
            return a_pv(ps, vt_ref, gg, chk)

        tl, chk = run_units(len(units), qk, sm, pv, fillers, slots or [0] * len(units), chk, DEPTH_A)
        tiles = dict(zip(units, tl))
        cols = []
        for gg in range(4):
            for e in range(2):
                cols.append(jnp.concatenate(
                    [tiles[(ii, s, gg)][64 * e:64 * e + 64] for ii in range(2) for s in range(2)], axis=0))
        return jnp.concatenate(cols, axis=1), chk

    def b_qk(i, g, nkb, dep=None):
        r0 = _mult(i * 128, 128)
        qt = q_s[1, i, g * 128:(g + 1) * 128, :]
        if nkb < 3:
            kw = k_s[1, g, pl.ds(_mult(r0 + KPAD - (nkb - 1) * 128, 16), nkb * 128), :]
            return _dot(kw, head_weights(qt))
        kr = k_s.at[1, g, pl.ds(_mult(r0 + KPAD - 256, 16), 384), :]
        qu = pltpu.bitcast(qt, u32)
        k0 = pltpu.bitcast(kr[0:64], u32)
        k2 = pltpu.roll(pltpu.bitcast(kr[320:384], u32), DH, axis=1)
        extra = []
        for h in range(4):
            lhs = pltpu.bitcast(jnp.where(lane_head32 == h, k0, k2), bf16)
            qh = qu[16 * h:16 * h + 16]
            blocks = [None] * 4
            blocks[h] = jnp.where(lane16 < 64, qh, zero16)
            blocks[(h + 1) % 4] = jnp.where(lane16 >= 64, qh, zero16)
            extra.append(_dot(lhs, stack_rows(blocks)))
        km = kr[64:320]
        if dep is not None and DEPK >= 0:
            ku = pltpu.bitcast(km[16 * DEPK:16 * DEPK + 16], u32) | (dep & zero_s[...])
            km = jnp.concatenate([x for x in (km[:16 * DEPK] if DEPK > 0 else None, pltpu.bitcast(ku, bf16),
                                              km[16 * DEPK + 16:] if DEPK < 15 else None) if x is not None], axis=0)
        main = _dot(km, head_weights(qt))
        return main, extra

    def b_sm(sT, nkb):
        ps = []
        dep = None
        for h in range(4):
            if nkb == 3:
                sh = sT[0][:, h * 128:(h + 1) * 128]
                ex = sT[1][h]
                c = jnp.concatenate([jnp.where(le[0:64], sh[192:256], ex),
                                     jnp.where(le[64:128], ex, sh[0:64])], axis=0)
                s1 = sh[64:192]
                pc = jnp.exp2(c)
                p1 = jnp.exp2(s1)
                acc8 = _fold8(pc + p1)
                au = pltpu.bitcast(acc8, u32)
                dep = au if dep is None else (dep | au)
                l = jnp.sum(acc8, axis=0, keepdims=True)
                pb = jnp.concatenate([jnp.where(le, 0.0, pc), p1, jnp.where(le, pc, 0.0)], axis=0)
            elif nkb == 2:
                sh = sT[:, h * 128:(h + 1) * 128]
                pc = jnp.where(le, jnp.exp2(sh[128:256]), 0.0)
                p1 = jnp.exp2(sh[0:128])
                l = jnp.sum(_fold8(pc + p1), axis=0, keepdims=True)
                pb = jnp.concatenate([p1, pc], axis=0)
            else:
                sh = sT[:, h * 128:(h + 1) * 128]
                pb = jnp.where(le, jnp.exp2(sh), 0.0)
                l = jnp.sum(_fold8(pb), axis=0, keepdims=True)
            ps.append((pb.astype(bf16), l))
        return ps, dep

    def b_pv(ps, i, g, nkb, chk):
        outs = []
        for h in range(4):
            hs = slice((g * 4 + h) * DH, (g * 4 + h + 1) * DH)
            pb, l = ps[h]
            vt = jnp.concatenate([vt_s[1, i - (nkb - 1) + tt, hs, :] for tt in range(nkb)], axis=1)
            o = _dot(vt, pb) * _recip(l)
            chk = (jnp.minimum(chk[0], l), jnp.maximum(chk[1], l), chk[2] + _fold8(o))
            outs.append(o)
        return jnp.concatenate(outs, axis=0).T.astype(bf16), chk

    def attn_b(t, chk, first=False, fillers=(), slots=None):
        units = [(t * 2 + ii, g, (ii + 1) if first else 3) for g in range(8) for ii in range(2)]

        def qk(n, dep):
            return b_qk(*units[n], dep=dep)

        def sm(n, sT):
            return b_sm(sT, units[n][2])

        def pv(n, ps, chk):
            i, g, nkb = units[n]
            return b_pv(ps, i, g, nkb, chk)

        tiles, chk = run_units(len(units), qk, sm, pv, fillers, slots or [0] * len(units), chk, DEPTH_B)
        lhs = jnp.concatenate([jnp.concatenate(tiles[2 * g:2 * g + 2], axis=0) for g in range(8)], axis=1)
        return lhs, chk

    def outproj(br, t, lhs, n=1):
        w = D // n
        for c in range(n):
            out_v[br, pl.ds(_mult(t * T, T), T), c * w:(c + 1) * w] = _dot(lhs, wo_v[br, :, c * w:(c + 1) * w]).astype(bf16)
            out_copy(br, t, c, n).start()

    def chk_init():
        return (jnp.full((1, 128), 1.0, f32), jnp.full((1, 128), 1.0, f32), jnp.zeros((8, 128), f32))

    def chk_bad(chk):
        lmin = jnp.min(chk[0])
        lmax = jnp.max(chk[1])
        tot = jnp.sum(chk[2])
        good = (lmin >= L_LO) & (lmax <= L_HI) & (jnp.abs(tot) <= 3.0e38)
        return jnp.logical_not(good)

    slots_a = [0] * 16
    slots_b = [0] * 16

    for f in proj_tasks(0, 0, 0, first=True):
        f()
    for kt in range(8):
        for p in range(4):
            woa_copy(kt, p).wait()

    def step_a(s, chk):
        br = (s + 1) // NT
        t = (s + 1) % NT
        pltpu.make_async_copy(xa_hbm.at[0, pl.ds(0, T), :], x_v.at[0, pl.ds(0, T), :], sem_x.at[s + 1]).wait()

        @pl.when(s < NT - 2)
        def _():
            x_copy(0, s + 2).start()

        @pl.when(s == NT - 3)
        def _():
            x_copy(1, 0).start()
            x_copy(1, 1).start()

        @pl.when(s == 1)
        def _():
            wb_copy().start()

        @pl.when(s == 4)
        def _():
            wob_copy().start()

        @pl.when(s == NT - 1)
        def _():
            wb_copy().wait()

        @pl.when(s == NT)
        def _():
            x_copy(1, 2).start()

        lhs, chk = attn_a(s - 1, chk, proj_tasks(br, t, (s + 1) * (T // 128)), slots_a)
        outproj(0, s - 1, lhs)
        return chk

    chk_a = lax.fori_loop(1, NT + 1, step_a, chk_init())

    wob_copy().wait()
    x_copy(1, 2).wait()
    x_copy(1, 3).start()
    lhs, chk_b = attn_b(0, chk_init(), True, proj_tasks(1, 2, None), slots_b)
    outproj(1, 0, lhs)

    def step_b(t, chk):
        pltpu.make_async_copy(xb_hbm.at[0, pl.ds(0, T), :], x_v.at[1, pl.ds(0, T), :], sem_x.at[NT + t + 2]).wait()

        @pl.when(t < NT - 3)
        def _():
            x_copy(1, t + 3).start()

        lhs, chk = attn_b(t, chk, False, proj_tasks(1, t + 2, None), slots_b)
        outproj(1, t, lhs)
        return chk

    chk_b = lax.fori_loop(1, NT - 2, step_b, chk_b)

    lhs, chk_b = attn_b(NT - 2, chk_b)
    outproj(1, NT - 2, lhs)
    lhs, chk_b = attn_b(NT - 1, chk_b)
    outproj(1, NT - 1, lhs, OSPLIT)
    bad_a = chk_bad(chk_a)
    bad_b = chk_bad(chk_b)
    for br in range(2):
        for t in range(NT):
            if br == 1 and t == NT - 1:
                for c in range(OSPLIT):
                    out_copy(br, t, c, OSPLIT).wait()
            else:
                out_copy(br, t).wait()

    def redo_outproj(br):
        def body(t, carry):
            r0 = pl.multiple_of(t * T, T)
            lhs = jnp.concatenate([o_s[kt, pl.ds(r0, T), :] for kt in range(8)], axis=1)
            out_v[br, pl.ds(r0, T), :] = _dot(lhs, wo_v[br]).astype(bf16)
            cp = pltpu.make_async_copy(out_v.at[br, pl.ds(r0, T), :], out_hbm.at[0, pl.ds(r0, T), pl.ds(br * D, D)],
                                       sem_out.at[br * NT + t])
            cp.start()
            cp.wait()
            return carry
        lax.fori_loop(0, NT, body, 0)

    @pl.when(bad_a)
    def _():
        def body(u, carry):
            j = u // 4
            gg = u % 4
            i = j // 2
            s = j % 2
            j64 = pl.multiple_of(j * 64, 64)
            bias = bias_a[jnp.minimum(j, 1)]

            def fin(s_static, vt_ref):
                ps = a_sm(a_qk(i, s_static, gg), bias, True)
                tile, _ = a_pv(ps, vt_ref, gg, None)
                o_s[2 * gg, pl.ds(j64, 64), :] = tile[0:64]
                o_s[2 * gg + 1, pl.ds(j64, 64), :] = tile[64:128]

            pl.when(s == 0)(lambda: fin(0, vsh_s.at[i]))
            pl.when(s == 1)(lambda: fin(1, vt_s.at[0, i]))
            return carry
        lax.fori_loop(0, 2 * NB * 4, body, 0)
        redo_outproj(0)

    @pl.when(bad_b)
    def _():
        def body(u, carry):
            i = u // 8
            g = u % 8
            kb = jnp.maximum(i - 2, 0)
            r0 = pl.multiple_of(i * 128, 128)
            qt = q_s[1, i, pl.ds(pl.multiple_of(g * 128, 128), 128), :]
            kw = k_s[1, g, pl.ds(pl.multiple_of(kb * 128 + KPAD, 16), 384), :]
            sT = _dot(kw, head_weights(qt))
            dpos = (_iota((384, 128), 1) + i * 128) - (_iota((384, 128), 0) + kb * 128)
            valid = (dpos >= 0) & (dpos < 256)
            outs = []
            for h in range(4):
                s = jnp.where(valid, sT[:, h * 128:(h + 1) * 128], NEG)
                p = jnp.exp2(s - jnp.max(s, axis=0, keepdims=True))
                l = jnp.sum(p, axis=0, keepdims=True)
                hs = pl.ds(pl.multiple_of((g * 4 + h) * DH, DH), DH)
                vt = jnp.concatenate([vt_s[1, kb + tt, hs, :] for tt in range(3)], axis=1)
                outs.append(_dot(vt, p.astype(bf16)) / l)
            o_s[g, pl.ds(r0, 128), :] = jnp.concatenate(outs, axis=0).T.astype(bf16)
            return carry
        lax.fori_loop(0, NB * 8, body, 0)
        redo_outproj(1)


def _call(A_x, A_wqkv, A_wo, B_x, B_wqkv, B_wo, interpret=False):
    any_spec = pl.BlockSpec(memory_space=pl.ANY)
    return pl.pallas_call(
        _kernel,
        out_shape=jax.ShapeDtypeStruct((1, S, 2 * D), bf16),
        in_specs=[any_spec] * 6,
        out_specs=any_spec,
        scratch_shapes=[
            pltpu.VMEM((2, S, D), bf16),
            pltpu.VMEM((2, D, 3 * D), bf16),
            pltpu.VMEM((2, D, D), bf16),
            pltpu.VMEM((2, NB, D, 128), bf16),
            pltpu.VMEM((2, 8, KPAD + S, 128), bf16),
            pltpu.VMEM((2, NB, D, 128), bf16),
            pltpu.VMEM((NB + 4, D, 128), bf16),
            pltpu.VMEM((64, D), f32),
            pltpu.VMEM((8, S, 128), bf16),
            pltpu.VMEM((2, S, D), bf16),
            pltpu.VMEM((2, 80, 128), f32),
            pltpu.VMEM((8, 128), u32),
            pltpu.SemaphoreType.DMA((2 * NT,)),
            pltpu.SemaphoreType.DMA((NCH,)),
            pltpu.SemaphoreType.DMA((1,)),
            pltpu.SemaphoreType.DMA((2,)),
            pltpu.SemaphoreType.DMA((2 * NT + 3,)),
        ],
        compiler_params=pltpu.CompilerParams(vmem_limit_bytes=100 * 1024 * 1024, disable_semaphore_checks=True),
        interpret=interpret,
    )(A_x, A_wqkv, A_wo, B_x, B_wqkv, B_wo)


@jax.jit
def pallas_concat_heads__sliding_local_dilated__sliding_block__prompt_kernel(A_x, A_wqkv, A_wo, B_x, B_wqkv, B_wo):
    return _call(A_x, A_wqkv, A_wo, B_x, B_wqkv, B_wo)
```

```python
import jax
import jax.numpy as jnp
from jax import lax
from jax.experimental import pallas as pl
from jax.experimental.pallas import tpu as pltpu

S = 2048
D = 1024
DH = 32
LOG2E = 1.4426950408889634
QSCALE = float(DH ** -0.5 * LOG2E)
NEG = float("-inf")
T = 256
NT = S // T
NB = S // 128
CW = 256
NCH = 3 * D // CW
L_LO = float(2.0 ** -60)
L_HI = float(2.0 ** 60)
DEPTH_B = 2
TIE_ROW = 4
FIRST_PARTS = (1, 0, 2)
WAIT_GROUPS = (1, 1, 2, 3, 5)
ISSUE = (1, 4, 7, 12, 12)
LAST_SPLIT = 2
f32 = jnp.float32
bf16 = jnp.bfloat16
u32 = jnp.uint32


def _dot(a, b):
    return jnp.dot(a, b, preferred_element_type=f32)


def _iota(shape, dim):
    return lax.broadcasted_iota(jnp.int32, shape, dim)


def _fold8(x):
    acc = x[0:8]
    for j in range(1, x.shape[0] // 8):
        acc = acc + x[8 * j:8 * j + 8]
    return acc


def _recip(l):
    r = pltpu.reciprocal(l, approx=True)
    return r * (2.0 - l * r)


def _mult(x, m):
    return x if isinstance(x, int) else pl.multiple_of(x, m)


def _kernel(xa_hbm, wa_hbm, woa_hbm, xb_hbm, wb_hbm, wob_hbm, out_hbm,
            x_v, w_v, wo_v, qt_s, k_s, kt_s, vt_s, o_s, out_v, zero_s,
            sem_x, sem_wa, sem_wb, sem_wo, sem_out):
    x_hbm = (xa_hbm, xb_hbm)

    def x_copy(br, t):
        r0 = _mult(t * T, T)
        return pltpu.make_async_copy(x_hbm[br].at[0, pl.ds(r0, T), :], x_v.at[br, pl.ds(r0, T), :],
                                     sem_x.at[br * NT + t])

    def x_wait(n):
        pltpu.make_async_copy(xa_hbm.at[0, pl.ds(0, T), :], x_v.at[0, pl.ds(0, T), :], sem_x.at[n]).wait()

    def wa_copy(c):
        return pltpu.make_async_copy(wa_hbm.at[:, pl.ds(c * CW, CW)], w_v.at[0, :, pl.ds(c * CW, CW)], sem_wa.at[c])

    def wb_copy():
        return pltpu.make_async_copy(wb_hbm, w_v.at[1], sem_wb.at[0])

    def wo_copy(br):
        return pltpu.make_async_copy((woa_hbm, wob_hbm)[br], wo_v.at[br], sem_wo.at[br])

    def out_copy(br, t, c=0, n=1):
        r0 = _mult(t * T, T)
        w = D // n
        return pltpu.make_async_copy(out_v.at[br, pl.ds(r0, T), pl.ds(c * w, w)],
                                     out_hbm.at[0, pl.ds(r0, T), pl.ds(br * D + c * w, w)],
                                     sem_out.at[br * NT + t + c])

    chunk_order = [c for part in FIRST_PARTS for c in range(part * D // CW, (part + 1) * D // CW)]
    starts = [sum(WAIT_GROUPS[:n]) for n in range(len(WAIT_GROUPS))]
    issued = [0]

    def issue_upto(k):
        while issued[0] < k:
            wa_copy(chunk_order[issued[0]]).start()
            issued[0] += 1

    def wait_chunk(c):
        pos = chunk_order.index(c)
        if pos not in starts:
            return
        n = starts.index(pos)
        if n == 0:
            x_copy(0, 0).wait()
            x_copy(0, 1).wait()
        for cc in chunk_order[pos:pos + WAIT_GROUPS[n]]:
            wa_copy(cc).wait()
        if n + 1 < len(WAIT_GROUPS):
            issue_upto(ISSUE[n + 1])
        else:
            x_copy(0, 2).start()
            wo_copy(0).start()

    x_copy(0, 0).start()
    issue_upto(ISSUE[0])
    x_copy(0, 1).start()
    zero_s[...] = jnp.zeros((8, 128), u32)

    def project(br, t, mode, first=False):
        rows = 2 * T if first else T
        r0 = _mult(t * T, T)
        t0 = t * (T // 128)
        kt0 = t0 if mode == "a" else t0 + br * NB
        kr0 = r0 if mode == "b" else _mult(br * r0 + (1 - br) * S, T)
        for part in (FIRST_PARTS if first else (2, 0, 1)):
            for c in range(D // CW):
                if first:
                    wait_chunk(part * D // CW + c)
                y = _dot(x_v[br, pl.ds(r0, rows), :], w_v[br, :, part * D + c * CW:part * D + (c + 1) * CW])
                cs = slice(c * CW, (c + 1) * CW)
                if part == 0:
                    y = y * QSCALE
                if part != 1 or mode != "b":
                    dst, d0 = (kt_s, kt0) if part == 1 else ((qt_s if part == 0 else vt_s).at[br], t0)
                    for tt in range(rows // 128):
                        dst[d0 + tt, cs, :] = y[tt * 128:(tt + 1) * 128, :].T.astype(bf16)
                if part == 1 and mode != "a":
                    yb = y.astype(bf16)
                    for g in range(CW // 128):
                        k_s[c * CW // 128 + g, pl.ds(kr0, rows), :] = yb[:, g * 128:(g + 1) * 128]

    sub8 = _iota((8, 128), 0)
    lane8 = _iota((8, 128), 1)
    lane16 = _iota((16, 128), 1)

    def unpack(u):
        return pltpu.bitcast(u << 16, f32), pltpu.bitcast(u & jnp.uint32(0xFFFF0000), f32)

    def round_hi(x):
        u = pltpu.bitcast(x, u32)
        return u + jnp.uint32(0x7FFF) + ((u >> 16) & jnp.uint32(1))

    def sublane_sums(xs):
        for dist in (4, 2, 1):
            m = (sub8 & dist) == 0
            half = len(xs) // 2
            if dist == 4:
                xs = [jnp.where(m, xs[n], xs[n + half]) + pltpu.roll(jnp.where(m, xs[n + half], xs[n]), 4, axis=0)
                      for n in range(half)]
            else:
                xs = [jnp.where(m, xs[n] + pltpu.roll(xs[n], 8 - dist, axis=0),
                                xs[n + half] + pltpu.roll(xs[n + half], dist, axis=0)) for n in range(half)]
        return xs[0]

    def a_head(t, h):
        hs = slice(h * DH, (h + 1) * DH)
        i0 = t * 2
        tiles = (jnp.maximum(i0 - 1, 0), i0, i0 + 1)
        ks = [pltpu.bitcast(kt_s[i, hs, :], u32) for i in tiles]
        vs = [pltpu.bitcast(vt_s[0, i, hs, :], u32) for i in tiles]
        kroll = [[x] + [pltpu.roll(x, 2 * w, axis=1) for w in range(1, 8)] for x in ks]
        vroll = [[x] + [pltpu.roll(x, 2 * w, axis=1) for w in range(1, 8)] for x in vs]
        outs = []
        for n in range(2):
            q_lo, q_hi = unpack(pltpu.bitcast(qt_s[0, i0 + n, hs, :], u32))

            def shifted(r, w):
                return r[n + 1][w] if w == 0 else jnp.where(lane16 < 2 * w, r[n][w], r[n + 1][w])

            parts = []
            for w in range(8):
                k_lo, k_hi = unpack(shifted(kroll, w))
                pr = q_lo * k_lo + q_hi * k_hi
                parts.append(pr[0:8] + pr[8:16])
            s = sublane_sums(parts)
            if n == 0:
                s = jnp.where(lane8 + i0 * 128 >= 2 * sub8, s, NEG)
            p = jnp.exp2(s - jnp.max(s, axis=0, keepdims=True))
            p = p * _recip(jnp.sum(p, axis=0, keepdims=True))
            o_lo = o_hi = None
            for w in range(8):
                v_lo, v_hi = unpack(shifted(vroll, w))
                pw = jnp.broadcast_to(p[w:w + 1], (16, 128))
                o_lo = pw * v_lo if o_lo is None else o_lo + pw * v_lo
                o_hi = pw * v_hi if o_hi is None else o_hi + pw * v_hi
            outs.append((round_hi(o_lo) >> 16) | (round_hi(o_hi) & jnp.uint32(0xFFFF0000)))
        return outs

    def attn_a(t):
        cols = []
        for g in range(8):
            heads = [a_head(t, 4 * g + h) for h in range(4)]
            cols.append(jnp.concatenate(
                [pltpu.bitcast(jnp.concatenate([hd[n] for hd in heads], axis=0), bf16).T for n in range(2)], axis=0))
        return jnp.concatenate(cols, axis=1)

    lane_head32 = _iota((32, 128), 1) // DH
    le = _iota((128, 128), 0) <= _iota((128, 128), 1)
    zero16 = jnp.zeros((16, 128), u32)

    def stack_rows(blocks):
        return pltpu.bitcast(jnp.concatenate([zero16 if b is None else b for b in blocks], axis=0), bf16)

    def head_weights(qt):
        qu = pltpu.bitcast(qt, u32)
        return jnp.concatenate(
            [stack_rows([qu[16 * h:16 * h + 16] if hh == h else None for hh in range(4)]) for h in range(4)], axis=1)

    def b_qk(i, g, nkb, tie):
        r0 = _mult(i * 128, 128)
        qt = qt_s[1, i, g * 128:(g + 1) * 128, :]
        if nkb < 3:
            return _dot(k_s[g, r0 - (nkb - 1) * 128:r0 + 128, :], head_weights(qt))
        kr = k_s.at[g, pl.ds(_mult(r0 - 256, 128), 384), :]
        qu = pltpu.bitcast(qt, u32)
        k0 = pltpu.bitcast(kr[0:64], u32)
        k2 = pltpu.roll(pltpu.bitcast(kr[320:384], u32), DH, axis=1)
        extra = []
        for h in range(4):
            lhs = pltpu.bitcast(jnp.where(lane_head32 == h, k0, k2), bf16)
            qh = qu[16 * h:16 * h + 16]
            blocks = [None] * 4
            blocks[h] = jnp.where(lane16 < 64, qh, zero16)
            blocks[(h + 1) % 4] = jnp.where(lane16 >= 64, qh, zero16)
            extra.append(_dot(lhs, stack_rows(blocks)))
        km = kr[64:320]
        if tie is not None:
            lo, hi = 16 * TIE_ROW, 16 * TIE_ROW + 16
            ku = pltpu.bitcast(km[lo:hi], u32) | (tie & zero_s[...])
            km = jnp.concatenate([km[:lo], pltpu.bitcast(ku, bf16), km[hi:]], axis=0)
        return _dot(km, head_weights(qt)), extra

    def b_probs(sT, nkb):
        ps = []
        tie = None
        for h in range(4):
            if nkb == 3:
                sh = sT[0][:, h * 128:(h + 1) * 128]
                ex = sT[1][h]
                pc = jnp.exp2(jnp.concatenate([jnp.where(le[0:64], sh[192:256], ex),
                                               jnp.where(le[64:128], ex, sh[0:64])], axis=0))
                p1 = jnp.exp2(sh[64:192])
                acc = _fold8(pc + p1)
                au = pltpu.bitcast(acc, u32)
                tie = au if tie is None else (tie | au)
                pb = jnp.concatenate([jnp.where(le, 0.0, pc), p1, jnp.where(le, pc, 0.0)], axis=0)
            elif nkb == 2:
                sh = sT[:, h * 128:(h + 1) * 128]
                pc = jnp.where(le, jnp.exp2(sh[128:256]), 0.0)
                p1 = jnp.exp2(sh[0:128])
                acc = _fold8(pc + p1)
                pb = jnp.concatenate([p1, pc], axis=0)
            else:
                pb = jnp.where(le, jnp.exp2(sT[:, h * 128:(h + 1) * 128]), 0.0)
                acc = _fold8(pb)
            ps.append((pb.astype(bf16), jnp.sum(acc, axis=0, keepdims=True)))
        return ps, tie

    def b_pv(ps, i, g, nkb, chk):
        outs = []
        for h in range(4):
            hs = slice((g * 4 + h) * DH, (g * 4 + h + 1) * DH)
            pb, l = ps[h]
            vt = jnp.concatenate([vt_s[1, i - (nkb - 1) + tt, hs, :] for tt in range(nkb)], axis=1)
            o = _dot(vt, pb) * _recip(l)
            chk = (jnp.minimum(chk[0], l), jnp.maximum(chk[1], l), chk[2] + _fold8(o))
            outs.append(o)
        return jnp.concatenate(outs, axis=0).T.astype(bf16), chk

    def attn_b(t, chk, first=False):
        units = [(t * 2 + ii, g, (ii + 1) if first else 3) for g in range(8) for ii in range(2)]
        sts = [b_qk(*units[n], None) for n in range(DEPTH_B)]
        tiles = []
        for n in range(len(units)):
            ps, tie = b_probs(sts[n], units[n][2])
            if n + DEPTH_B < len(units):
                sts.append(b_qk(*units[n + DEPTH_B], tie))
            tile, chk = b_pv(ps, *units[n], chk)
            tiles.append(tile)
        return jnp.concatenate([jnp.concatenate(tiles[2 * g:2 * g + 2], axis=0) for g in range(8)], axis=1), chk

    def outproj(br, t, lhs, n=1):
        w = D // n
        for c in range(n):
            out_v[br, pl.ds(_mult(t * T, T), T), c * w:(c + 1) * w] = _dot(
                lhs, wo_v[br, :, c * w:(c + 1) * w]).astype(bf16)
            out_copy(br, t, c, n).start()

    project(0, 0, "a", first=True)
    wo_copy(0).wait()

    def step_a(s, carry):
        x_wait(s + 1)

        @pl.when(s < NT - 2)
        def _():
            x_copy(0, s + 2).start()

        @pl.when(s == NT - 3)
        def _():
            x_copy(1, 0).start()
            x_copy(1, 1).start()

        @pl.when(s == 1)
        def _():
            wb_copy().start()

        @pl.when(s == 4)
        def _():
            wo_copy(1).start()

        @pl.when(s == NT - 1)
        def _():
            wb_copy().wait()

        @pl.when(s == NT)
        def _():
            x_copy(1, 2).start()

        lhs = attn_a(s - 1)
        project((s + 1) // NT, (s + 1) % NT, "ab")
        outproj(0, s - 1, lhs)
        return carry

    lax.fori_loop(1, NT + 1, step_a, 0)

    wo_copy(1).wait()
    x_copy(1, 2).wait()
    x_copy(1, 3).start()
    chk = (jnp.full((1, 128), 1.0, f32), jnp.full((1, 128), 1.0, f32), jnp.zeros((8, 128), f32))
    lhs, chk = attn_b(0, chk, first=True)
    project(1, 2, "b")
    outproj(1, 0, lhs)

    def step_b(t, chk):
        x_wait(NT + t + 2)

        @pl.when(t < NT - 3)
        def _():
            x_copy(1, t + 3).start()

        lhs, chk = attn_b(t, chk)
        project(1, t + 2, "b")
        outproj(1, t, lhs)
        return chk

    chk = lax.fori_loop(1, NT - 2, step_b, chk)

    lhs, chk = attn_b(NT - 2, chk)
    outproj(1, NT - 2, lhs)
    lhs, chk = attn_b(NT - 1, chk)
    outproj(1, NT - 1, lhs, LAST_SPLIT)
    safe = (jnp.min(chk[0]) >= L_LO) & (jnp.max(chk[1]) <= L_HI) & (jnp.abs(jnp.sum(chk[2])) <= 3.0e38)
    for br in range(2):
        for t in range(NT - br):
            out_copy(br, t).wait()
    for c in range(LAST_SPLIT):
        out_copy(1, NT - 1, c, LAST_SPLIT).wait()

    @pl.when(jnp.logical_not(safe))
    def _():
        def attn(u, carry):
            i = u // 8
            g = u % 8
            kb = jnp.maximum(i - 2, 0)
            qt = qt_s[1, i, pl.ds(pl.multiple_of(g * 128, 128), 128), :]
            sT = _dot(k_s[g, pl.ds(pl.multiple_of(kb * 128, 128), 384), :], head_weights(qt))
            dpos = (_iota((384, 128), 1) + i * 128) - (_iota((384, 128), 0) + kb * 128)
            valid = (dpos >= 0) & (dpos < 256)
            outs = []
            for h in range(4):
                s = jnp.where(valid, sT[:, h * 128:(h + 1) * 128], NEG)
                p = jnp.exp2(s - jnp.max(s, axis=0, keepdims=True))
                l = jnp.sum(p, axis=0, keepdims=True)
                hs = pl.ds(pl.multiple_of((g * 4 + h) * DH, DH), DH)
                vt = jnp.concatenate([vt_s[1, kb + tt, hs, :] for tt in range(3)], axis=1)
                outs.append(_dot(vt, p.astype(bf16)) / l)
            o_s[g, pl.ds(pl.multiple_of(i * 128, 128), 128), :] = jnp.concatenate(outs, axis=0).T.astype(bf16)
            return carry

        lax.fori_loop(0, NB * 8, attn, 0)

        def proj(t, carry):
            r0 = pl.multiple_of(t * T, T)
            lhs = jnp.concatenate([o_s[kt, pl.ds(r0, T), :] for kt in range(8)], axis=1)
            out_v[1, pl.ds(r0, T), :] = _dot(lhs, wo_v[1]).astype(bf16)
            cp = out_copy(1, t)
            cp.start()
            cp.wait()
            return carry

        lax.fori_loop(0, NT, proj, 0)


@jax.jit
def pallas_concat_heads__sliding_local_dilated__sliding_block__prompt_kernel(
    A_x: jax.Array,
    A_wqkv: jax.Array,
    A_wo: jax.Array,
    B_x: jax.Array,
    B_wqkv: jax.Array,
    B_wo: jax.Array,
):
    any_spec = pl.BlockSpec(memory_space=pl.ANY)
    return pl.pallas_call(
        _kernel,
        out_shape=jax.ShapeDtypeStruct((1, S, 2 * D), bf16),
        in_specs=[any_spec] * 6,
        out_specs=any_spec,
        scratch_shapes=[
            pltpu.VMEM((2, S, D), bf16),
            pltpu.VMEM((2, D, 3 * D), bf16),
            pltpu.VMEM((2, D, D), bf16),
            pltpu.VMEM((2, NB, D, 128), bf16),
            pltpu.VMEM((8, S + T, 128), bf16),
            pltpu.VMEM((NB + 4, D, 128), bf16),
            pltpu.VMEM((2, NB, D, 128), bf16),
            pltpu.VMEM((8, S, 128), bf16),
            pltpu.VMEM((2, S, D), bf16),
            pltpu.VMEM((8, 128), u32),
            pltpu.SemaphoreType.DMA((2 * NT,)),
            pltpu.SemaphoreType.DMA((NCH,)),
            pltpu.SemaphoreType.DMA((1,)),
            pltpu.SemaphoreType.DMA((2,)),
            pltpu.SemaphoreType.DMA((2 * NT + LAST_SPLIT - 1,)),
        ],
        compiler_params=pltpu.CompilerParams(vmem_limit_bytes=100 * 1024 * 1024),
    )(A_x, A_wqkv, A_wo, B_x, B_wqkv, B_wo)
```
